```python
import jax
import jax.numpy as jnp

def _softmax(x, axis=-1):
    return jax.nn.softmax(x, axis=axis)

def _gelu(x):
    return jax.nn.gelu(x, approximate=True)

def _silu(x):
    return jax.nn.silu(x)

def _sigmoid(x):
    return jax.nn.sigmoid(x)

def _layernorm(x, axis=-1, eps=1e-05):
    m = jnp.mean(x, axis=axis, keepdims=True)
    v = jnp.var(x, axis=axis, keepdims=True)
    return (x - m) / jnp.sqrt(v + eps)

def _scatter_add(tgt, idx, src, axis=0):
    return tgt.at[idx].add(src)

def _segment_sum(src, seg, n):
    return jax.ops.segment_sum(src, seg, n)

class _Rng:

    def __init__(self, key):
        self._k = key

    def _next(self):
        self._k, sub = jax.random.split(self._k)
        return sub

    def normal(self, shape):
        return jax.random.normal(self._next(), shape, dtype=jnp.bfloat16)

    def randint(self, lo, hi, shape):
        return jax.random.randint(self._next(), shape, lo, hi, dtype=jnp.int32)

    def uniform(self, shape, lo=0.0, hi=1.0):
        return jax.random.uniform(self._next(), shape, jnp.bfloat16, lo, hi)

    def permutation(self, n):
        return jax.random.permutation(self._next(), n)
kernel_name = 'interleave_layers__linear_kernel_hedgehog__mixer_gmlp__prompt'

def _fwd_setup_inputs():
    _rng = _Rng(jax.random.key(int.from_bytes(__import__("os").urandom(4), "little")))
    _w = lambda a: (lambda t: t.astype(jnp.bfloat16) if jnp.issubdtype(t.dtype, jnp.floating) else t)(jnp.asarray(a))

    def _A_setup():
        B, S, D, H = (1, 2048, 640, 32)
        Dh = D // H
        return {'x': _w((lambda *s: _rng.normal(s) * 0.05)(B, S, D)), 'wqkv': _w((lambda *s: _rng.normal(s) * 0.05)(D, 3 * D)), 'w_phi': _w((lambda *s: _rng.normal(s) * 0.05)(H, Dh, Dh) * Dh ** (-0.5)), 'wo': _w((lambda *s: _rng.normal(s) * 0.05)(D, D))}
    _A_in = _A_setup()

    def _B_setup():
        B, S, D, F = (1, 2048, 640, 1536)
        Fh = F // 2
        return {'x': _w((lambda *s: _rng.normal(s) * 0.05)(B, S, D)), 'w_in': _w((lambda *s: _rng.normal(s) * 0.05)(D, 2 * Fh)), 'w_sp': _w(0.01 * (lambda *s: _rng.normal(s) * 0.05)(S, S)), 'b_sp': _w(1.0 + 0.01 * (lambda *s: _rng.normal(s) * 0.05)(S)), 'w_out': _w((lambda *s: _rng.normal(s) * 0.05)(Fh, D))}
    _B_in = _B_setup()
    return {'A_x': _A_in['x'], 'A_wqkv': _A_in['wqkv'], 'A_w_phi': _A_in['w_phi'], 'A_wo': _A_in['wo'], 'B_x': _B_in['x'], 'B_w_in': _B_in['w_in'], 'B_w_sp': _B_in['w_sp'], 'B_b_sp': _B_in['b_sp'], 'B_w_out': _B_in['w_out']}

def _fwd_reference(A_x, A_wqkv, A_w_phi, A_wo, B_x, B_w_in, B_w_sp, B_b_sp, B_w_out):

    def _A_ref(x, wqkv, w_phi, wo):
        B, S, D = x.shape
        H = 32
        Dh = D // H
        qkv = (lambda x, *d: x.transpose(*d))((x @ wqkv).reshape(B, S, 3, H, Dh), 2, 0, 3, 1, 4)
        q, k, v = (qkv[0], qkv[1], qkv[2])
        pq = jnp.einsum('bhsd,hdf->bhsf', q, w_phi)
        pk = jnp.einsum('bhsd,hdf->bhsf', k, w_phi)
        phi_q = jnp.concatenate([_softmax(pq, axis=-1), _softmax(-pq, axis=-1)], axis=-1)
        phi_k = jnp.concatenate([_softmax(pk, axis=-1), _softmax(-pk, axis=-1)], axis=-1)
        kv = jnp.einsum('bhsf,bhsd->bhfd', phi_k, v)
        z = jnp.einsum('bhsf->bhf', phi_k)
        num = jnp.einsum('bhqf,bhfd->bhqd', phi_q, kv)
        den = jnp.einsum('bhqf,bhf->bhq', phi_q, z)[..., None] + 1e-06
        o = num / den
        return (lambda x, *d: x.transpose(*d))(o, 0, 2, 1, 3).reshape(B, S, D) @ wo

    def _B_ref(x, w_in, w_sp, b_sp, w_out):
        B, S, D = x.shape
        F = w_in.shape[-1]
        Fh = F // 2
        z = _gelu(jnp.einsum('bsd,df->bsf', x, w_in))
        z1 = z[..., :Fh].copy()
        z2 = _layernorm(z[..., Fh:], axis=-1)
        g = jnp.einsum('ts,bsf->btf', w_sp, z2) + b_sp[None, :, None]
        return jnp.einsum('bsf,fd->bsd', z1 * g, w_out)
    x = A_x
    x = x + _A_ref(_layernorm(x, axis=-1), A_wqkv, A_w_phi, A_wo)
    x = x + _B_ref(_layernorm(x, axis=-1), B_w_in, B_w_sp, B_b_sp, B_w_out)
    x = x + _A_ref(_layernorm(x, axis=-1), A_wqkv, A_w_phi, A_wo)
    x = x + _B_ref(_layernorm(x, axis=-1), B_w_in, B_w_sp, B_b_sp, B_w_out)
    return x

def setup_inputs():
    _inp = _fwd_setup_inputs()
    _gk = jax.random.fold_in(jax.random.key(int.from_bytes(__import__("os").urandom(4), "little")), 2 ** 31 - 1)
    _shapes = [[1, 2048, 640]]
    _dtypes = ['bfloat16']
    _gks = jax.random.split(_gk, len(_shapes))
    _gs = [jax.random.normal(k, s, dtype=jnp.dtype(d)) * 0.05 for k, s, d in zip(_gks, _shapes, _dtypes)]
    _inp['grad_out'] = _gs[0]
    return _inp

def reference(A_x, A_wqkv, A_w_phi, A_wo, B_w_in, B_w_sp, B_b_sp, B_w_out, B_x, grad_out):
    _const = dict(B_x=B_x)

    def _f(*_d):
        return _fwd_reference(**{'A_x': _d[0], 'A_wqkv': _d[1], 'A_w_phi': _d[2], 'A_wo': _d[3], 'B_w_in': _d[4], 'B_w_sp': _d[5], 'B_b_sp': _d[6], 'B_w_out': _d[7], **_const})
    _out, _vjp = jax.vjp(_f, A_x, A_wqkv, A_w_phi, A_wo, B_w_in, B_w_sp, B_b_sp, B_w_out)
    _grads = _vjp(grad_out)
    _out0 = jnp.asarray(_out)
    return (_out0, *[jnp.asarray(_g) for _g in _grads])
```

```python
import math

import jax
import jax.numpy as jnp
from jax import lax
import jax.experimental.pallas as pl
import jax.experimental.pallas.tpu as pltpu

S, D, H, DH, FH = 2048, 640, 32, 20, 768
NG, GR = 8, 80
PR, VR = 160, 96
TS = 256
NT = S // TS
F32, BF16 = jnp.float32, jnp.bfloat16
C0 = math.sqrt(2.0 / math.pi)
C1 = 0.044715


def _mm(a, b):
    return jnp.dot(a, b, preferred_element_type=F32)


def _mmt(a, b):
    return lax.dot_general(a, b, (((1,), (1,)), ((), ())), preferred_element_type=F32)


def _iota(shape, dim):
    return lax.broadcasted_iota(jnp.int32, shape, dim)


def _perm_parts(r):
    g = (r * 820) >> 16
    return g * 4 + (r & 3), (r - g * 80) >> 2


def _orig_parts(c):
    h = (c * 3277) >> 16
    return h, c - h * 20


def _csum(x):
    return jnp.sum(x, axis=0, keepdims=True)


def _ln_fwd(x, n):
    mu = _csum(x) * (1.0 / n)
    xc = x - mu
    rstd = lax.rsqrt(_csum(xc * xc) * (1.0 / n) + 1e-5)
    return xc * rstd, rstd


def _ln_bwd(dh, h, rstd, n):
    m1 = _csum(dh) * (1.0 / n)
    m2 = _csum(dh * h) * (1.0 / n)
    return (dh - m1 - h * m2) * rstd


def _half_swap(x):
    return pltpu.roll(x, 4, 0)


def _phi(p):
    t = p.shape[-1]
    p3 = p.reshape(10, 8, t)
    mx = jnp.max(p3, axis=0)
    mx = jnp.maximum(mx, _half_swap(mx))
    mn = jnp.min(p3, axis=0)
    mn = jnp.minimum(mn, _half_swap(mn))
    e1 = jnp.exp(p3 - mx[None])
    e2 = jnp.exp(mn[None] - p3)
    s1 = jnp.sum(e1, axis=0)
    s2 = jnp.sum(e2, axis=0)
    r1 = 1.0 / (s1 + _half_swap(s1))
    r2 = 1.0 / (s2 + _half_swap(s2))
    return jnp.concatenate([(e1 * r1[None]).reshape(GR, t), (e2 * r2[None]).reshape(GR, t)], axis=0)


def _phi_bwd(phi, dphi):
    t = phi.shape[-1]
    ph = phi.astype(F32).reshape(20, 8, t)
    w = ph * dphi.reshape(20, 8, t)
    s1 = jnp.sum(w[:10], axis=0)
    s2 = jnp.sum(w[10:], axis=0)
    s1 = s1 + _half_swap(s1)
    s2 = s2 + _half_swap(s2)
    return ((w[:10] - ph[:10] * s1[None]) - (w[10:] - ph[10:] * s2[None])).reshape(GR, t)


def _gelu_and_grad(a):
    a2 = a * a
    t = jnp.tanh(a * (C0 + (C0 * C1) * a2))
    hp = 0.5 + 0.5 * t
    z = a * hp
    dz = hp + z * (1.0 - t) * (C0 + (3.0 * C0 * C1) * a2)
    return z, dz


def _kernel(x_hbm, wqkv_hbm, wphi_ref, wo_hbm, win_hbm, wsp_hbm, bsp_ref, wout_hbm, gout_hbm,
            out_hbm, gx_hbm, dwqkv_hbm, dwphi_ref, dwo_hbm, dwin_hbm, dwsp_hbm, dbsp_ref, dwout_hbm,
            X, STG, WSP, WQKV, WO, WIN, WOUT, BDT, PM, HA, PQ, PK, VP, O, HB, DG, Z1, Z2, GG,
            RA, RB, R2, RD, KV, KVT, sem):

    def tile(j):
        return pl.ds(pl.multiple_of(j * TS, TS), TS)

    cp_x = pltpu.make_async_copy(x_hbm, STG, sem.at[0])
    cp_wqkv = pltpu.make_async_copy(wqkv_hbm, WQKV, sem.at[1])
    cp_wo = pltpu.make_async_copy(wo_hbm, WO, sem.at[2])
    cp_win = pltpu.make_async_copy(win_hbm, WIN, sem.at[3])
    cp_wsp = pltpu.make_async_copy(wsp_hbm, WSP, sem.at[4])
    cp_wout = pltpu.make_async_copy(wout_hbm, WOUT, sem.at[5])
    for c in (cp_wqkv, cp_x, cp_wo, cp_win, cp_wout, cp_wsp):
        c.start()

    def get_ft():
        _, fd = _perm_parts(_iota((D, 128), 0))
        return jnp.where(fd == _iota((D, 128), 1), 1.0, 0.0).astype(BF16)

    for m in range(0, D, 128):
        rh, rd = _perm_parts(_iota((128, D), 0) + m)
        ch, cd = _orig_parts(_iota((128, D), 1))
        same = rh == ch
        PM[m:m + 128, :] = jnp.where(same & (rd == cd), 1.0, 0.0).astype(BF16)
        BDT[m:m + 128, :] = jnp.where(same, _mmt(get_ft()[m:m + 128], wphi_ref[...]), 0.0).astype(BF16)

    def get_kvmask():
        return ((_iota((PR, 128), 0) & 3) == (_iota((PR, 128), 1) & 3)) & (_iota((PR, 128), 1) < 88)

    ones_rows = jnp.where(_iota((16, S), 0) < 8, 1.0, 0.0).astype(BF16)
    for l in range(2):
        for g in range(NG):
            VP[l, g, GR:VR, :] = ones_rows

    def load_T(j):
        return STG[tile(j), :].astype(F32).T

    def forward(WFT, WOT, WINT, WOUTT, KVA):
        cp_wqkv.wait()
        for k, L in enumerate((BDT, BDT, PM)):
            for m in range(0, D, 128):
                WFT[k * D + m:k * D + m + 128, :] = _mmt(L[m:m + 128, :], WQKV[:, k * D:(k + 1) * D]).astype(BF16)
        cp_wo.wait()
        for m in range(0, D, 128):
            WOT[m:m + 128, :] = _mm(PM[...], WO[:, m:m + 128]).T.astype(BF16)
        for m in range(0, D, 128):
            WO[m:m + 128, :] = WOT[:, m:m + 128].astype(F32).T.astype(BF16)
        cp_win.wait()
        for m in range(0, 2 * FH, 128):
            WINT[m:m + 128, :] = WIN[:, m:m + 128].astype(F32).T.astype(BF16)
        cp_wout.wait()
        for m in range(0, D, 128):
            WOUTT[m:m + 128, :] = WOUT[:, m:m + 128].astype(F32).T.astype(BF16)
        cp_x.wait()

        def xin(j, c):
            X[:, tile(j)] = load_T(j)
            return c
        lax.fori_loop(0, NT, xin, 0)
        cp_wsp.wait()

        def layer(l, c):
            KVA[...] = jnp.zeros(KVA.shape, F32)

            def f1(j, c):
                sl = tile(j)
                h, rstd = _ln_fwd(X[:, sl], D)
                h = h.astype(BF16)
                HA[l, :, sl] = h
                RA[l, :, sl] = rstd
                for g in range(NG):
                    w = jnp.concatenate([WFT[k * D + g * GR:k * D + (g + 1) * GR, :] for k in range(3)], axis=0)
                    p = _mm(w, h)
                    PQ[l, g, :, sl] = _phi(p[0:GR]).astype(BF16)
                    PK[l, g, :, sl] = _phi(p[GR:2 * GR]).astype(BF16)
                    VP[l, g, 0:GR, sl] = p[2 * GR:3 * GR].astype(BF16)
                    KVA[g, :, 0:VR] += _mmt(PK[l, g, :, sl], VP[l, g, :, sl])
                return c
            with jax.named_scope("F1"):
                lax.fori_loop(0, NT, f1, 0)
            for g in range(NG):
                kv = jnp.where(get_kvmask(), KVA[g], 0.0)
                KV[l, g] = kv.astype(BF16)
                KVT[l, g] = jnp.concatenate([kv, jnp.zeros((256 - PR, 128), F32)], axis=0).T.astype(BF16)

            def f2(j, c):
                sl = tile(j)
                for g in range(NG):
                    num = _mm(KVT[l, g, 0:VR, 0:PR], PQ[l, g, :, sl])
                    rden = 1.0 / (num[GR:GR + 8] + 1e-6)
                    RD[l, g * 8:(g + 1) * 8, sl] = rden
                    o = num[0:GR].reshape(10, 8, TS) * rden[None]
                    O[l, g * GR:(g + 1) * GR, sl] = o.reshape(GR, TS).astype(BF16)
                x = X[:, sl] + _mm(WOT[...], O[l, :, sl])
                X[:, sl] = x
                h, rstd = _ln_fwd(x, D)
                h = h.astype(BF16)
                HB[l, :, sl] = h
                RB[l, :, sl] = rstd
                z2 = []
                for m in range(0, 2 * FH, 128):
                    z, dz = _gelu_and_grad(_mm(WINT[m:m + 128, :], h))
                    GG[l, m:m + 128, sl] = dz.astype(BF16)
                    if m < FH:
                        Z1[l, m:m + 128, sl] = z.astype(BF16)
                    else:
                        z2.append(z)
                z2n, rstd2 = _ln_fwd(jnp.concatenate(z2, axis=0), FH)
                Z2[l, :, sl] = z2n.astype(BF16)
                R2[l, :, sl] = rstd2
                return c
            with jax.named_scope("F2"):
                lax.fori_loop(0, NT, f2, 0)

            def f3(j, c):
                sl = tile(j)
                gt = _mmt(Z2[l], WSP[sl, :]) + bsp_ref[:, sl].astype(F32)
                DG[l, :, sl] = gt.astype(BF16)
                u = (Z1[l, :, sl].astype(F32) * gt).astype(BF16)
                X[:, sl] += _mm(WOUTT[...], u)
                return c
            with jax.named_scope("F3"):
                lax.fori_loop(0, NT, f3, 0)
            return c
        lax.fori_loop(0, 2, layer, 0)

    pl.run_scoped(forward, pltpu.VMEM((3 * D, D), BF16), pltpu.VMEM((D, D), BF16),
                  pltpu.VMEM((2 * FH, D), BF16), pltpu.VMEM((D, FH), BF16),
                  pltpu.VMEM((NG, PR, 128), F32))

    def store_T_all(dst, s):
        def body(j, c):
            STG[tile(j), :] = X[:, tile(j)].T.astype(BF16)
            return c
        lax.fori_loop(0, NT, body, 0)
        cp = pltpu.make_async_copy(STG, dst, s)
        cp.start()
        cp.wait()

    store_T_all(out_hbm, sem.at[0])
    cp_g = pltpu.make_async_copy(gout_hbm, STG, sem.at[0])
    cp_g.start()
    cp_g.wait()

    def gin(j, c):
        X[:, tile(j)] = load_T(j)
        return c
    lax.fori_loop(0, NT, gin, 0)

    def backward(WF, DWF, DWO, DWIN, DWOUT, DGN, DP, DKVA, DBS):
        for k, L in enumerate((BDT, BDT, PM)):
            for m in range(0, D, 128):
                WF[m:m + 128, k * D:(k + 1) * D] = _mmt(WQKV[m:m + 128, k * D:(k + 1) * D], L[...]).astype(BF16)
        for r in (DWF, DWO, DWIN, DWOUT, DBS):
            r[...] = jnp.zeros(r.shape, F32)

        def layer(i, c):
            l = 1 - i
            DKVA[...] = jnp.zeros(DKVA.shape, F32)

            def b3(j, c):
                sl = tile(j)
                dy = X[:, sl].astype(BF16)
                du = _mm(WOUT[...], dy)
                z1 = Z1[l, :, sl].astype(F32)
                gt = DG[l, :, sl].astype(F32)
                DWOUT[...] += _mmt((z1 * gt).astype(BF16), dy)
                dg = du * z1
                DBS[:, sl] += _csum(dg)
                DG[l, :, sl] = dg.astype(BF16)
                DGN[l, sl, :] = dg.T.astype(BF16)
                GG[l, 0:FH, sl] = (du * gt * GG[l, 0:FH, sl].astype(F32)).astype(BF16)
                return c
            with jax.named_scope("B3"):
                lax.fori_loop(0, NT, b3, 0)

            def b2(j, c):
                sl = tile(j)
                dz = _mm(DG[l], WSP[:, sl])
                dz = _ln_bwd(dz, Z2[l, :, sl].astype(F32), R2[l, :, sl], FH)
                GG[l, FH:2 * FH, sl] = (dz * GG[l, FH:2 * FH, sl].astype(F32)).astype(BF16)
                da = GG[l, :, sl]
                hb = HB[l, :, sl]
                for m in range(0, 2 * FH, 256):
                    DWIN[:, m:m + 256] += _mmt(hb, GG[l, m:m + 256, sl])
                dx = X[:, sl] + _ln_bwd(_mm(WIN[...], da), hb.astype(F32), RB[l, :, sl], D)
                X[:, sl] = dx
                dy = dx.astype(BF16)
                DWO[...] += _mmt(O[l, :, sl], dy)
                for g in range(NG):
                    do = _mm(WO[g * GR:(g + 1) * GR, :], dy).reshape(10, 8, TS)
                    dnum = do * RD[l, g * 8:(g + 1) * 8, sl][None]
                    o = O[l, g * GR:(g + 1) * GR, sl].astype(F32).reshape(10, 8, TS)
                    dden = -jnp.sum(dnum * o, axis=0)
                    dn = jnp.concatenate([dnum.reshape(GR, TS), dden, jnp.zeros((8, TS), F32)], axis=0).astype(BF16)
                    phq = PQ[l, g, :, sl]
                    DKVA[g, :, 0:VR] += _mmt(phq, dn)
                    dpq = _phi_bwd(phq, _mm(KV[l, g, :, 0:VR], dn))
                    PQ[l, g, 0:GR, sl] = dpq.astype(BF16)
                return c
            with jax.named_scope("B2"):
                lax.fori_loop(0, NT, b2, 0)
            for g in range(NG):
                kv = jnp.where(get_kvmask(), DKVA[g], 0.0)
                KV[l, g] = kv.astype(BF16)
                KVT[l, g] = jnp.concatenate([kv, jnp.zeros((256 - PR, 128), F32)], axis=0).T.astype(BF16)

            def b1(j, c):
                sl = tile(j)
                for g in range(NG):
                    phk = PK[l, g, :, sl]
                    DP[g * GR:(g + 1) * GR, :] = PQ[l, g, 0:GR, sl]
                    dpk = _phi_bwd(phk, _mm(KV[l, g, :, 0:VR], VP[l, g, :, sl]))
                    DP[D + g * GR:D + (g + 1) * GR, :] = dpk.astype(BF16)
                    DP[2 * D + g * GR:2 * D + (g + 1) * GR, :] = _mm(KVT[l, g, 0:GR, 0:PR], phk).astype(BF16)
                ha = HA[l, :, sl]
                dp = DP[...]
                for m in range(0, 3 * D, 128):
                    DWF[:, m:m + 128] += _mmt(ha, DP[m:m + 128, :])
                X[:, sl] += _ln_bwd(_mm(WF[...], dp), ha.astype(F32), RA[l, :, sl], D)
                return c
            with jax.named_scope("B1"):
                lax.fori_loop(0, NT, b1, 0)
            return c
        lax.fori_loop(0, 2, layer, 0)

        store_T_all(gx_hbm, sem.at[0])
        dbsp_ref[...] = DBS[...].astype(BF16)

        def wsp_grad(j, c):
            sl = tile(j)
            WSP[:, sl] = (_mm(DGN[0], Z2[0, :, sl]) + _mm(DGN[1], Z2[1, :, sl])).astype(BF16)
            return c
        with jax.named_scope("DWSP"):
            lax.fori_loop(0, NT, wsp_grad, 0)

        WF[...] = DWF[...].astype(BF16)
        for m in range(0, D, 128):
            acc = 0.0
            for k in range(2):
                w = WQKV[:, k * D + m:k * D + m + 128].astype(F32).T.astype(BF16)
                acc = acc + _mm(w, WF[:, k * D:(k + 1) * D])
            oh, _ = _orig_parts(_iota((128, D), 0) + m)
            ph, _ = _perm_parts(_iota((128, D), 1))
            dwphi_ref[m:m + 128, :] = _mm(jnp.where(oh == ph, acc, 0.0).astype(BF16), get_ft()).astype(BF16)
        for k, L in enumerate((BDT, BDT, PM)):
            for m in range(0, D, 128):
                WQKV[m:m + 128, k * D:(k + 1) * D] = _mm(WF[m:m + 128, k * D:(k + 1) * D], L[...]).astype(BF16)
        WO[...] = DWO[...].astype(BF16)
        for m in range(0, D, 128):
            BDT[m:m + 128, :] = _mm(PM[:, m:m + 128].astype(F32).T.astype(BF16), WO[...]).astype(BF16)
        WIN[...] = DWIN[...].astype(BF16)
        WOUT[...] = DWOUT[...].astype(BF16)
        cps = [pltpu.make_async_copy(a, b, sem.at[i]) for i, (a, b) in enumerate(
            [(WQKV, dwqkv_hbm), (BDT, dwo_hbm), (WIN, dwin_hbm), (WSP, dwsp_hbm), (WOUT, dwout_hbm)])]
        for c in cps:
            c.start()
        for c in cps:
            c.wait()

    pl.run_scoped(backward, pltpu.VMEM((D, 3 * D), BF16), pltpu.VMEM((D, 3 * D), F32),
                  pltpu.VMEM((D, D), F32), pltpu.VMEM((D, 2 * FH), F32), pltpu.VMEM((FH, D), F32),
                  pltpu.VMEM((2, S, FH), BF16), pltpu.VMEM((3 * D, TS), BF16),
                  pltpu.VMEM((NG, PR, 128), F32), pltpu.VMEM((1, S), F32))


@jax.jit
def pallas_interleave_layers__linear_kernel_hedgehog__mixer_gmlp__prompt_kernel(
        A_x, A_wqkv, A_w_phi, A_wo, B_x, B_w_in, B_w_sp, B_b_sp, B_w_out, grad_out):
    del B_x
    hbm = pl.BlockSpec(memory_space=pl.ANY)
    vm = pl.BlockSpec(memory_space=pltpu.VMEM)
    sds = jax.ShapeDtypeStruct
    V = pltpu.VMEM
    wphi = jnp.pad(A_w_phi.reshape(D, DH), ((0, 0), (0, 128 - DH)))
    outs = pl.pallas_call(
        _kernel,
        in_specs=[hbm, hbm, vm, hbm, hbm, hbm, vm, hbm, hbm],
        out_specs=[hbm, hbm, hbm, vm, hbm, hbm, hbm, vm, hbm],
        out_shape=[sds((S, D), BF16), sds((S, D), BF16), sds((D, 3 * D), BF16), sds((D, 128), BF16),
                   sds((D, D), BF16), sds((D, 2 * FH), BF16), sds((S, S), BF16), sds((1, S), BF16),
                   sds((FH, D), BF16)],
        scratch_shapes=[
            V((D, S), F32), V((S, D), BF16), V((S, S), BF16), V((D, 3 * D), BF16), V((D, D), BF16),
            V((D, 2 * FH), BF16), V((FH, D), BF16), V((D, D), BF16), V((D, D), BF16),
            V((2, D, S), BF16), V((2, NG, PR, S), BF16), V((2, NG, PR, S), BF16), V((2, NG, VR, S), BF16),
            V((2, D, S), BF16), V((2, D, S), BF16), V((2, FH, S), BF16), V((2, FH, S), BF16),
            V((2, FH, S), BF16), V((2, 2 * FH, S), BF16),
            V((2, 1, S), F32), V((2, 1, S), F32), V((2, 1, S), F32), V((2, 64, S), F32),
            V((2, NG, PR, 128), BF16), V((2, NG, 128, 256), BF16),
            pltpu.SemaphoreType.DMA((6,)),
        ],
        compiler_params=pltpu.CompilerParams(vmem_limit_bytes=127 * 1024 * 1024),
    )(A_x.reshape(S, D), A_wqkv, wphi, A_wo, B_w_in, B_w_sp, B_b_sp.reshape(1, S), B_w_out,
      grad_out.reshape(S, D))
    out, gx, dwqkv, dwphi, dwo, dwin, dwsp, dbsp, dwout = outs
    return (out.reshape(1, S, D), gx.reshape(1, S, D), dwqkv, dwphi[:, :DH].reshape(H, DH, DH), dwo,
            dwin, dwsp, dbsp.reshape(S), dwout)
```

```python
import math

import jax
import jax.numpy as jnp
from jax import lax
import jax.experimental.pallas as pl
import jax.experimental.pallas.tpu as pltpu

S, D, H, DH, FH = 2048, 640, 32, 20, 768
NG, GR = 8, 80
PR, VR = 160, 96
TS = 256
NT = S // TS
F32, BF16 = jnp.float32, jnp.bfloat16
C0 = math.sqrt(2.0 / math.pi)
C1 = 0.044715


def _mm(a, b):
    return jnp.dot(a, b, preferred_element_type=F32)


def _mmt(a, b):
    return lax.dot_general(a, b, (((1,), (1,)), ((), ())), preferred_element_type=F32)


def _iota(shape, dim):
    return lax.broadcasted_iota(jnp.int32, shape, dim)


def _perm_parts(r):
    g = (r * 820) >> 16
    return g * 4 + (r & 3), (r - g * 80) >> 2


def _orig_parts(c):
    h = (c * 3277) >> 16
    return h, c - h * 20


def _krange(m):
    lo, hi = (m // GR) * GR, ((m + 127) // GR + 1) * GR
    return (lo // 128) * 128, min(D, -(-hi // 128) * 128)


def _csum(x):
    return jnp.sum(x, axis=0, keepdims=True)


def _ln_fwd(x, n):
    mu = _csum(x) * (1.0 / n)
    xc = x - mu
    rstd = lax.rsqrt(_csum(xc * xc) * (1.0 / n) + 1e-5)
    return xc * rstd, rstd


def _ln_bwd(dh, h, rstd, n):
    m1 = _csum(dh) * (1.0 / n)
    m2 = _csum(dh * h) * (1.0 / n)
    return (dh - m1 - h * m2) * rstd


def _half_swap(x):
    return pltpu.roll(x, 4, 0)


def _phi(p):
    t = p.shape[-1]
    p3 = p.reshape(10, 8, t)
    mx = jnp.max(p3, axis=0)
    mx = jnp.maximum(mx, _half_swap(mx))
    mn = jnp.min(p3, axis=0)
    mn = jnp.minimum(mn, _half_swap(mn))
    e1 = jnp.exp(p3 - mx[None])
    e2 = jnp.exp(mn[None] - p3)
    s1 = jnp.sum(e1, axis=0)
    s2 = jnp.sum(e2, axis=0)
    r1 = 1.0 / (s1 + _half_swap(s1))
    r2 = 1.0 / (s2 + _half_swap(s2))
    return jnp.concatenate([(e1 * r1[None]).reshape(GR, t), (e2 * r2[None]).reshape(GR, t)], axis=0)


def _phi_bwd(phi, dphi):
    t = phi.shape[-1]
    ph = phi.astype(F32).reshape(20, 8, t)
    w = ph * dphi.reshape(20, 8, t)
    s1 = jnp.sum(w[:10], axis=0)
    s2 = jnp.sum(w[10:], axis=0)
    s1 = s1 + _half_swap(s1)
    s2 = s2 + _half_swap(s2)
    return ((w[:10] - ph[:10] * s1[None]) - (w[10:] - ph[10:] * s2[None])).reshape(GR, t)


def _gelu_and_grad(a):
    a2 = a * a
    t = jnp.tanh(a * (C0 + (C0 * C1) * a2))
    hp = 0.5 + 0.5 * t
    z = a * hp
    dz = hp + z * (1.0 - t) * (C0 + (3.0 * C0 * C1) * a2)
    return z, dz


def _kernel(x_hbm, wqkv_hbm, wphi_ref, wo_hbm, win_hbm, wsp_hbm, bsp_ref, wout_hbm, gout_hbm,
            out_hbm, gx_hbm, dwqkv_hbm, dwphi_ref, dwo_hbm, dwin_hbm, dwsp_hbm, dbsp_ref, dwout_hbm,
            X, STG, WSP, WQKV, WO, WIN, WOUT, BDT, PM, HA, PQ, PK, VP, O, HB, DG, Z1, Z2, GG,
            RA, RB, R2, RD, KV, KVT, DGN, sem):

    def tile(j):
        return pl.ds(pl.multiple_of(j * TS, TS), TS)

    cp_x = pltpu.make_async_copy(x_hbm, STG, sem.at[0])
    cp_wqkv = pltpu.make_async_copy(wqkv_hbm, WQKV, sem.at[1])
    cp_wo = pltpu.make_async_copy(wo_hbm, WO, sem.at[2])
    cp_win = pltpu.make_async_copy(win_hbm, WIN, sem.at[3])
    cp_wsp = pltpu.make_async_copy(wsp_hbm, WSP, sem.at[4])
    cp_wout = pltpu.make_async_copy(wout_hbm, WOUT, sem.at[5])
    cp_g = pltpu.make_async_copy(gout_hbm, DGN.at[0, :, 0:D], sem.at[6])
    for c in (cp_wqkv, cp_x):
        c.start()

    def get_ft():
        _, fd = _perm_parts(_iota((D, 128), 0))
        return jnp.where(fd == _iota((D, 128), 1), 1.0, 0.0).astype(BF16)

    for m in range(0, D, 128):
        rh, rd = _perm_parts(_iota((128, D), 0) + m)
        ch, cd = _orig_parts(_iota((128, D), 1))
        same = rh == ch
        PM[m:m + 128, :] = jnp.where(same & (rd == cd), 1.0, 0.0).astype(BF16)
        BDT[m:m + 128, :] = jnp.where(same, _mmt(get_ft()[m:m + 128], wphi_ref[...]), 0.0).astype(BF16)

    def get_kvmask():
        return ((_iota((PR, 128), 0) & 3) == (_iota((PR, 128), 1) & 3)) & (_iota((PR, 128), 1) < 88)

    ones_rows = jnp.where(_iota((16, S), 0) < 8, 1.0, 0.0).astype(BF16)
    for l in range(2):
        for g in range(NG):
            VP[l, g, GR:VR, :] = ones_rows

    def load_T(j):
        return STG[tile(j), :].astype(F32).T

    def forward(WFT, WOT, WINT, WOUTT, KVA, ZT):
        cp_wqkv.wait()
        for c in (cp_wo, cp_win, cp_wout):
            c.start()
        for k, L in enumerate((BDT, BDT, PM)):
            for m in range(0, D, 128):
                a, b = _krange(m)
                WFT[k * D + m:k * D + m + 128, :] = _mmt(L[m:m + 128, a:b], WQKV[:, k * D + a:k * D + b]).astype(BF16)
        cp_wo.wait()
        for m in range(0, D, 128):
            WOT[m:m + 128, :] = _mm(PM[...], WO[:, m:m + 128]).T.astype(BF16)
        for m in range(0, D, 128):
            WO[m:m + 128, :] = WOT[:, m:m + 128].astype(F32).T.astype(BF16)
        cp_win.wait()
        for m in range(0, 2 * FH, 128):
            WINT[m:m + 128, :] = WIN[:, m:m + 128].astype(F32).T.astype(BF16)
        cp_wout.wait()
        for m in range(0, D, 128):
            WOUTT[m:m + 128, :] = WOUT[:, m:m + 128].astype(F32).T.astype(BF16)
        cp_x.wait()
        cp_wsp.start()
        cp_g.start()

        def xin(j, c):
            X[:, tile(j)] = load_T(j)
            return c
        lax.fori_loop(0, NT, xin, 0)

        def layer(l, c):
            KVA[...] = jnp.zeros(KVA.shape, F32)

            def ln_a(j):
                sl = tile(j)
                h, rstd = _ln_fwd(X[:, sl], D)
                HA[l, :, sl] = h.astype(BF16)
                RA[l, :, sl] = rstd

            def f1(j, c):
                sl = tile(j)
                h = HA[l, :, sl]

                def pmm(k, g):
                    return _mm(WFT[k * D + g * GR:k * D + (g + 1) * GR, :], h)
                pq = pmm(0, 0)
                for g in range(NG):
                    pk = pmm(1, g)
                    PQ[l, g, :, sl] = _phi(pq).astype(BF16)
                    v = pmm(2, g)
                    if g + 1 < NG:
                        pq = pmm(0, g + 1)
                    PK[l, g, :, sl] = _phi(pk).astype(BF16)
                    VP[l, g, 0:GR, sl] = v.astype(BF16)
                    if g == 3:
                        ln_a(jnp.minimum(j + 1, NT - 1))
                    if g > 0:
                        KVA[g - 1, :, 0:VR] += _mmt(PK[l, g - 1, :, sl], VP[l, g - 1, :, sl])
                KVA[NG - 1, :, 0:VR] += _mmt(PK[l, NG - 1, :, sl], VP[l, NG - 1, :, sl])
                return c
            with jax.named_scope("F1"):
                ln_a(0)
                lax.fori_loop(0, NT, f1, 0)
            for g in range(NG):
                kv = jnp.where(get_kvmask(), KVA[g], 0.0)
                KV[l, g] = kv.astype(BF16)
                KVT[l, g] = jnp.concatenate([kv, jnp.zeros((256 - PR, 128), F32)], axis=0).T.astype(BF16)

            def f2_attn(j):
                sl = tile(j)
                nums = [None] * NG
                nums[0] = _mm(KVT[l, 0, 0:VR, 0:PR], PQ[l, 0, :, sl])
                for g in range(NG):
                    if g + 1 < NG:
                        nums[g + 1] = _mm(KVT[l, g + 1, 0:VR, 0:PR], PQ[l, g + 1, :, sl])
                    num = nums[g]
                    rden = 1.0 / (num[GR:GR + 8] + 1e-6)
                    RD[l, g * 8:(g + 1) * 8, sl] = rden
                    o = num[0:GR].reshape(10, 8, TS) * rden[None]
                    O[l, g * GR:(g + 1) * GR, sl] = o.reshape(GR, TS).astype(BF16)
                X[:, sl] += _mm(WOT[...], O[l, :, sl])

            def f2_ln(j):
                sl = tile(j)
                h, rstd = _ln_fwd(X[:, sl], D)
                HB[l, :, sl] = h.astype(BF16)
                RB[l, :, sl] = rstd

            def f2_mlp(j, mid1, mid2):
                sl = tile(j)
                h = HB[l, :, sl]
                order = list(range(FH, 2 * FH, 128)) + list(range(0, FH, 128))
                nxt = _mm(WINT[order[0]:order[0] + 128, :], h)
                for i, m in enumerate(order):
                    a = nxt
                    if i + 1 < len(order):
                        nxt = _mm(WINT[order[i + 1]:order[i + 1] + 128, :], h)
                    z, dz = _gelu_and_grad(a)
                    GG[l, m:m + 128, sl] = dz.astype(BF16)
                    if m < FH:
                        Z1[l, m:m + 128, sl] = z.astype(BF16)
                    else:
                        ZT[m - FH:m - FH + 128, :] = z
                    if i == 5:
                        mid1()
                        z2n, rstd2 = _ln_fwd(ZT[...], FH)
                        Z2[l, :, sl] = z2n.astype(BF16)
                        R2[l, :, sl] = rstd2
                    if i == 8:
                        mid2()

            def f2(j, c):
                f2_mlp(j, lambda: f2_attn(j + 1), lambda: f2_ln(j + 1))
                return c
            with jax.named_scope("F2"):
                f2_attn(0)
                f2_ln(0)
                lax.fori_loop(0, NT - 1, f2, 0)
                f2_mlp(NT - 1, lambda: None, lambda: None)

            pl.when(l == 0)(cp_wsp.wait)

            def f3(j, c):
                sl = tile(j)
                gt = _mmt(Z2[l], WSP[sl, :]) + bsp_ref[:, sl].astype(F32)
                DG[l, :, sl] = gt.astype(BF16)
                u = (Z1[l, :, sl].astype(F32) * gt).astype(BF16)
                X[:, sl] += _mm(WOUTT[...], u)
                return c
            with jax.named_scope("F3"):
                lax.fori_loop(0, NT, f3, 0)
            return c
        lax.fori_loop(0, 2, layer, 0)

    pl.run_scoped(forward, pltpu.VMEM((3 * D, D), BF16), pltpu.VMEM((D, D), BF16),
                  pltpu.VMEM((2 * FH, D), BF16), pltpu.VMEM((D, FH), BF16),
                  pltpu.VMEM((NG, PR, 128), F32), pltpu.VMEM((FH, TS), F32))

    def store_T_all(dst, s):
        def body(j, c):
            STG[tile(j), :] = X[:, tile(j)].T.astype(BF16)
            return c
        lax.fori_loop(0, NT, body, 0)
        cp = pltpu.make_async_copy(STG, dst, s)
        cp.start()
        return cp

    cp_out = store_T_all(out_hbm, sem.at[0])
    cp_g.wait()

    def gin(j, c):
        X[:, tile(j)] = DGN[0, tile(j), 0:D].astype(F32).T
        return c
    lax.fori_loop(0, NT, gin, 0)

    def backward(WF, DWF, DWO, DWIN, DWOUT, DP, DKVA, DBS):
        for k, L in enumerate((BDT, BDT, PM)):
            for m in range(0, D, 128):
                a, b = _krange(m)
                WF[:, k * D + m:k * D + m + 128] = _mmt(WQKV[:, k * D + a:k * D + b], L[m:m + 128, a:b]).astype(BF16)
        for r in (DWF, DWO, DWIN, DWOUT, DBS):
            r[...] = jnp.zeros(r.shape, F32)

        cp_dwo = pltpu.make_async_copy(WO, dwo_hbm, sem.at[2])
        cp_dwin = pltpu.make_async_copy(WIN, dwin_hbm, sem.at[3])
        cp_dwout = pltpu.make_async_copy(WOUT, dwout_hbm, sem.at[5])

        def cp_dwsp(j):
            return pltpu.make_async_copy(WSP.at[:, tile(j)], dwsp_hbm.at[:, tile(j)], sem.at[4])

        def layer(i, c):
            l = 1 - i
            DKVA[...] = jnp.zeros(DKVA.shape, F32)

            def b3(j, c):
                sl = tile(j)
                dy = X[:, sl].astype(BF16)
                du = _mm(WOUT[...], dy)
                z1 = Z1[l, :, sl].astype(F32)
                gt = DG[l, :, sl].astype(F32)
                DWOUT[...] += _mmt((z1 * gt).astype(BF16), dy)
                dg = du * z1
                DBS[:, sl] += _csum(dg)
                DG[l, :, sl] = dg.astype(BF16)
                DGN[l, sl, :] = dg.T.astype(BF16)
                GG[l, 0:FH, sl] = (du * gt * GG[l, 0:FH, sl].astype(F32)).astype(BF16)
                return c
            with jax.named_scope("B3"):
                lax.fori_loop(0, NT, b3, 0)

            def b2(j, c):
                sl = tile(j)
                hb = HB[l, :, sl]
                dz = _mm(DG[l], WSP[:, sl])
                for m in range(0, FH, 256):
                    DWIN[:, m:m + 256] += _mmt(hb, GG[l, m:m + 256, sl])
                dz = _ln_bwd(dz, Z2[l, :, sl].astype(F32), R2[l, :, sl], FH)
                GG[l, FH:2 * FH, sl] = (dz * GG[l, FH:2 * FH, sl].astype(F32)).astype(BF16)
                dh = _mm(WIN[...], GG[l, :, sl])
                for m in range(FH, 2 * FH, 256):
                    DWIN[:, m:m + 256] += _mmt(hb, GG[l, m:m + 256, sl])
                dx = X[:, sl] + _ln_bwd(dh, hb.astype(F32), RB[l, :, sl], D)
                X[:, sl] = dx
                dy = dx.astype(BF16)
                dos = [None] * NG
                dos[0] = _mm(WO[0:GR, :], dy)
                pend = None
                for g in range(NG):
                    if g + 1 < NG:
                        dos[g + 1] = _mm(WO[(g + 1) * GR:(g + 2) * GR, :], dy)
                    dnum = dos[g].reshape(10, 8, TS) * RD[l, g * 8:(g + 1) * 8, sl][None]
                    o = O[l, g * GR:(g + 1) * GR, sl].astype(F32).reshape(10, 8, TS)
                    dden = -jnp.sum(dnum * o, axis=0)
                    dn = jnp.concatenate([dnum.reshape(GR, TS), dden, jnp.zeros((8, TS), F32)], axis=0).astype(BF16)
                    phq = PQ[l, g, :, sl]
                    dphi = _mm(KV[l, g, :, 0:VR], dn)
                    DKVA[g, :, 0:VR] += _mmt(phq, dn)
                    r = slice(g * GR, (g + 1) * GR)
                    DWO[r, :] += _mmt(O[l, r, sl], dy)
                    PQ[l, g, 0:GR, sl] = _phi_bwd(phq, dphi).astype(BF16)
                return c
            with jax.named_scope("B2"):
                lax.fori_loop(0, NT, b2, 0)

            @pl.when(l == 0)
            def _():
                WOUT[...] = DWOUT[...].astype(BF16)
                cp_dwout.start()
                WIN[...] = DWIN[...].astype(BF16)
                cp_dwin.start()
                dbsp_ref[...] = DBS[...].astype(BF16)
                for m in range(0, D, 128):
                    a, b = _krange(m)
                    WO[m:m + 128, :] = _mm(PM[a:b, m:m + 128].astype(F32).T.astype(BF16),
                                           DWO[a:b, :].astype(BF16)).astype(BF16)
                cp_dwo.start()

                def wsp_grad(j, c):
                    sl = tile(j)
                    WSP[:, sl] = (_mm(DGN[0], Z2[0, :, sl]) + _mm(DGN[1], Z2[1, :, sl])).astype(BF16)
                    cp_dwsp(j).start()
                    return c
                with jax.named_scope("DWSP"):
                    lax.fori_loop(0, NT, wsp_grad, 0)
            for g in range(NG):
                kv = jnp.where(get_kvmask(), DKVA[g], 0.0)
                KV[l, g] = kv.astype(BF16)
                KVT[l, g] = jnp.concatenate([kv, jnp.zeros((256 - PR, 128), F32)], axis=0).T.astype(BF16)

            def b1(j, c):
                sl = tile(j)
                ha = HA[l, :, sl]
                dphi = _mm(KV[l, 0, :, 0:VR], VP[l, 0, :, sl])
                for g in range(NG):
                    DP[g * GR:(g + 1) * GR, :] = PQ[l, g, 0:GR, sl]
                for g in range(NG):
                    phk = PK[l, g, :, sl]
                    cur = dphi
                    DP[2 * D + g * GR:2 * D + (g + 1) * GR, :] = _mm(KVT[l, g, 0:GR, 0:PR], phk).astype(BF16)
                    if g + 1 < NG:
                        dphi = _mm(KV[l, g + 1, :, 0:VR], VP[l, g + 1, :, sl])
                    if g < 5:
                        DWF[:, g * 128:(g + 1) * 128] += _mmt(ha, DP[g * 128:(g + 1) * 128, :])
                    DP[D + g * GR:D + (g + 1) * GR, :] = _phi_bwd(phk, cur).astype(BF16)
                dh = _mm(WF[...], DP[...])
                for m in range(D, 3 * D, 128):
                    DWF[:, m:m + 128] += _mmt(ha, DP[m:m + 128, :])
                X[:, sl] += _ln_bwd(dh, ha.astype(F32), RA[l, :, sl], D)
                return c
            with jax.named_scope("B1"):
                lax.fori_loop(0, NT, b1, 0)
            return c
        lax.fori_loop(0, 2, layer, 0)

        cp_out.wait()
        cp_gx = store_T_all(gx_hbm, sem.at[0])
        WF[...] = DWF[...].astype(BF16)
        for m in range(0, D, 128):
            a, b = _krange(m)
            acc = 0.0
            for k in range(2):
                w = WQKV[:, k * D + m:k * D + m + 128].astype(F32).T.astype(BF16)
                acc = acc + _mm(w, WF[:, k * D + a:k * D + b])
            oh, _ = _orig_parts(_iota((128, b - a), 0) + m)
            ph, _ = _perm_parts(_iota((128, b - a), 1) + a)
            dwphi_ref[m:m + 128, :] = _mm(jnp.where(oh == ph, acc, 0.0).astype(BF16), get_ft()[a:b]).astype(BF16)
        for k, L in enumerate((BDT, BDT, PM)):
            for m in range(0, D, 128):
                a, b = _krange(m)
                WQKV[:, k * D + m:k * D + m + 128] = _mm(WF[:, k * D + a:k * D + b], L[a:b, m:m + 128]).astype(BF16)
        cp_dwqkv = pltpu.make_async_copy(WQKV, dwqkv_hbm, sem.at[1])
        cp_dwqkv.start()
        for c in (cp_dwout, cp_dwin, cp_dwo, cp_gx, cp_dwqkv):
            c.wait()
        for j in range(NT):
            cp_dwsp(j).wait()

    pl.run_scoped(backward, pltpu.VMEM((D, 3 * D), BF16), pltpu.VMEM((D, 3 * D), F32),
                  pltpu.VMEM((D, D), F32), pltpu.VMEM((D, 2 * FH), F32), pltpu.VMEM((FH, D), F32),
                  pltpu.VMEM((3 * D, TS), BF16),
                  pltpu.VMEM((NG, PR, 128), F32), pltpu.VMEM((1, S), F32))


def _kernel_outer(*refs):
    V = pltpu.VMEM
    pl.run_scoped(lambda *scr: _kernel(*refs, *scr),
            V((D, S), F32), V((S, D), BF16), V((S, S), BF16), V((D, 3 * D), BF16), V((D, D), BF16),
            V((D, 2 * FH), BF16), V((FH, D), BF16), V((D, D), BF16), V((D, D), BF16),
            V((2, D, S), BF16), V((2, NG, PR, S), BF16), V((2, NG, PR, S), BF16), V((2, NG, VR, S), BF16),
            V((2, D, S), BF16), V((2, D, S), BF16), V((2, FH, S), BF16), V((2, FH, S), BF16),
            V((2, FH, S), BF16), V((2, 2 * FH, S), BF16),
            V((2, 1, S), F32), V((2, 1, S), F32), V((2, 1, S), F32), V((2, 64, S), F32),
            V((2, NG, PR, 128), BF16), V((2, NG, 128, 256), BF16), V((2, S, FH), BF16),
            pltpu.SemaphoreType.DMA((7,)),
        )


@jax.jit
def pallas_interleave_layers__linear_kernel_hedgehog__mixer_gmlp__prompt_kernel(
        A_x, A_wqkv, A_w_phi, A_wo, B_x, B_w_in, B_w_sp, B_b_sp, B_w_out, grad_out):
    del B_x
    hbm = pl.BlockSpec(memory_space=pl.ANY)
    vm = pl.BlockSpec(memory_space=pltpu.VMEM)
    sds = jax.ShapeDtypeStruct
    wphi = jnp.pad(A_w_phi.reshape(D, DH), ((0, 0), (0, 128 - DH)))
    outs = pl.pallas_call(
        _kernel_outer,
        in_specs=[hbm, hbm, vm, hbm, hbm, hbm, vm, hbm, hbm],
        out_specs=[hbm, hbm, hbm, vm, hbm, hbm, hbm, vm, hbm],
        out_shape=[sds((S, D), BF16), sds((S, D), BF16), sds((D, 3 * D), BF16), sds((D, 128), BF16),
                   sds((D, D), BF16), sds((D, 2 * FH), BF16), sds((S, S), BF16), sds((1, S), BF16),
                   sds((FH, D), BF16)],
        compiler_params=pltpu.CompilerParams(vmem_limit_bytes=127 * 1024 * 1024),
    )(A_x.reshape(S, D), A_wqkv, wphi, A_wo, B_w_in, B_w_sp, B_b_sp.reshape(1, S), B_w_out,
      grad_out.reshape(S, D))
    out, gx, dwqkv, dwphi, dwo, dwin, dwsp, dbsp, dwout = outs
    return (out.reshape(1, S, D), gx.reshape(1, S, D), dwqkv, dwphi[:, :DH].reshape(H, DH, DH), dwo,
            dwin, dwsp, dbsp.reshape(S), dwout)
```
